```python
import jax
import jax.numpy as jnp

def _softmax(x, axis=-1):
    return jax.nn.softmax(x, axis=axis)
def _gelu(x):
    return jax.nn.gelu(x, approximate=True)
def _silu(x):
    return jax.nn.silu(x)
def _sigmoid(x):
    return jax.nn.sigmoid(x)
def _layernorm(x, axis=-1, eps=1e-5):
    m = jnp.mean(x, axis=axis, keepdims=True)
    v = jnp.var(x, axis=axis, keepdims=True)
    return (x - m) / jnp.sqrt(v + eps)
def _scatter_add(tgt, idx, src, axis=0):
    return tgt.at[idx].add(src)
def _segment_sum(src, seg, n):
    return jax.ops.segment_sum(src, seg, n)
class _Rng:
    def __init__(self, key):
        self._k = key
    def _next(self):
        self._k, sub = jax.random.split(self._k)
        return sub
    def normal(self, shape):
        return jax.random.normal(self._next(), shape, dtype=jnp.bfloat16)
    def randint(self, lo, hi, shape):
        return jax.random.randint(self._next(), shape, lo, hi, dtype=jnp.int32)
    def uniform(self, shape, lo=0.0, hi=1.0):
        return jax.random.uniform(self._next(), shape, jnp.bfloat16, lo, hi)
    def permutation(self, n):
        return jax.random.permutation(self._next(), n)


kernel_name = 'parallel_sum__linear_attn_block__moe_arch_mod__prompt'

def setup_inputs():
    _rng = _Rng(jax.random.key(int.from_bytes(__import__("os").urandom(4), "little")))
    _w = (lambda a: (lambda t: t.astype(jnp.bfloat16) if jnp.issubdtype(t.dtype, jnp.floating) else t)(jnp.asarray(a)))
    def _A_setup():
        B, S, D = 1, 2048, 1024
        return {
            "x": _w((lambda *s: _rng.normal(s) * 0.05)(B, S, D)),
            "wqkv": _w((lambda *s: _rng.normal(s) * 0.05)(D, 3 * D)),
            "wo": _w((lambda *s: _rng.normal(s) * 0.05)(D, D)),
        }
    _A_in = _A_setup()

    def _B_setup():
        B, S, D, F, C = 1, 2048, 1024, 3584, 1
        return {
            "x": _w((lambda *s: _rng.normal(s) * 0.05)(B, S, D)),
            "w_r": _w((lambda *s: _rng.normal(s) * 0.05)(D)),
            "w_gate": _w((lambda *s: _rng.normal(s) * 0.05)(D, F)),
            "w_up": _w((lambda *s: _rng.normal(s) * 0.05)(D, F)),
            "w_down": _w((lambda *s: _rng.normal(s) * 0.05)(F, D)),
        }
    _B_in = _B_setup()

    return {
        "A_x": _A_in["x"],
        "A_wqkv": _A_in["wqkv"],
        "A_wo": _A_in["wo"],
        "B_x": _B_in["x"],
        "B_w_r": _B_in["w_r"],
        "B_w_gate": _B_in["w_gate"],
        "B_w_up": _B_in["w_up"],
        "B_w_down": _B_in["w_down"],
    }

def reference(A_x, A_wqkv, A_wo, B_x, B_w_r, B_w_gate, B_w_up, B_w_down):
    def _A_ref(x, wqkv, wo):
        B, S, D = x.shape
        H = 32; Dh = D // H
        qkv = (lambda x, *d: x.transpose(*d))((x @ wqkv).reshape(B, S, 3, H, Dh), 2, 0, 3, 1, 4)
        q, k, v = qkv[0], qkv[1], qkv[2]
        phi = lambda t: jnp.where(t > 0, t + 1, jnp.exp(t)) + 1e-6
        pq, pk = phi(q), phi(k)
        kv = jnp.einsum("bhsd,bhse->bhde", pk, v)
        z = jnp.einsum("bhsd->bhd", pk)
        num = jnp.einsum("bhqd,bhde->bhqe", pq, kv)
        den = jnp.einsum("bhqd,bhd->bhq", pq, z)[..., None] + 1e-6
        o = num / den
        return (lambda x, *d: x.transpose(*d))(o, 0, 2, 1, 3).reshape(B, S, D) @ wo

    def _B_ref(x, w_r, w_gate, w_up, w_down):
        B, S, D = x.shape
        C = 1
        r = x @ w_r
        idx = jnp.argsort(-r, axis=-1)[:, :C]
        idx_e = jnp.repeat(idx.reshape(B, C, 1), D, axis=2)
        x_sel = jnp.take_along_axis(x, idx_e, axis=1)
        g = _silu(x_sel @ w_gate)
        u = x_sel @ w_up
        y = (g * u) @ w_down
        r_sel = _sigmoid(jnp.take_along_axis(r, idx, axis=1))
        y = y * r_sel.reshape(B, C, 1)
        b_off = (jnp.arange(B) * S).reshape(B, 1)
        flat_idx = (idx + b_off).reshape(B * C)
        zero = (x * 0.0).reshape(B * S, D)
        upd = _scatter_add(zero, flat_idx, y.reshape(B * C, D), axis=0)
        return x + upd.reshape(B, S, D)

    x = A_x
    xn = _layernorm(x, axis=-1)
    return x + _A_ref(xn, A_wqkv, A_wo) + _B_ref(xn, B_w_r, B_w_gate, B_w_up, B_w_down)
```

```python
import functools

import jax
import jax.numpy as jnp
from jax import lax
import jax.experimental.pallas as pl
import jax.experimental.pallas.tpu as pltpu

F32 = jnp.float32
BF16 = jnp.bfloat16

H = 32
TM = 256
LN_EPS = 1e-5
PHI_EPS = 1e-6


def _phi(t):
    return jnp.where(t > 0, t + 1.0, jnp.exp(t)) + PHI_EPS


def _fused_kernel(x_hbm, wqkv_hbm, wo_hbm, wr_ref, wg_hbm, wu_hbm, wd_hbm, o_hbm,
                  x_v, xn_v, wq_v, wk_v, wv_v, wo_v, wg_v, wu_v, wd_v,
                  p_v, m_v, zb_v, o_v, xsem, wsem, osem, *, S, D, F):
    NB = S // TM
    Dh = D // H
    NG = D // 128

    def x_copy(i):
        return pltpu.make_async_copy(
            x_hbm.at[pl.ds(i * TM, TM), :], x_v.at[pl.ds(i * TM, TM), :], xsem.at[i])

    def o_copy(i):
        return pltpu.make_async_copy(
            o_v.at[pl.ds(i * TM, TM), :], o_hbm.at[pl.ds(i * TM, TM), :], osem.at[i])

    wq_c = pltpu.make_async_copy(wqkv_hbm.at[:, pl.ds(0, D)], wq_v, wsem.at[0])
    wk_c = pltpu.make_async_copy(wqkv_hbm.at[:, pl.ds(D, D)], wk_v, wsem.at[1])
    wv_c = pltpu.make_async_copy(wqkv_hbm.at[:, pl.ds(2 * D, D)], wv_v, wsem.at[2])
    wo_c = pltpu.make_async_copy(wo_hbm, wo_v, wsem.at[3])
    wg_c = pltpu.make_async_copy(wg_hbm, wg_v, wsem.at[4])
    wu_c = pltpu.make_async_copy(wu_hbm, wu_v, wsem.at[5])
    wd_c = pltpu.make_async_copy(wd_hbm, wd_v, wsem.at[6])

    x_copy(0).start()
    wk_c.start()
    for i in range(1, NB):
        x_copy(i).start()
    wq_c.start()
    wv_c.start()
    wo_c.start()
    wg_c.start()
    wu_c.start()
    wd_c.start()

    wr = wr_ref[...].astype(F32)

    def ln_block(i, best, bidx):
        r0 = pl.multiple_of(i * TM, TM)
        x = x_v[pl.ds(r0, TM), :].astype(F32)
        m = jnp.mean(x, axis=-1, keepdims=True)
        xc = x - m
        v = jnp.mean(xc * xc, axis=-1, keepdims=True)
        xn = (xc * lax.rsqrt(v + LN_EPS)).astype(BF16)
        xn_v[pl.ds(r0, TM), :] = xn
        r = jnp.sum(xn.astype(F32) * wr, axis=-1, keepdims=True)
        rows = lax.broadcasted_iota(jnp.int32, (TM, 1), 0) + r0
        upd = r > best
        return jnp.where(upd, r, best), jnp.where(upd, rows, bidx)

    wk_c.wait()

    def p1_body(i, carry):
        best, bidx, z = carry
        x_copy(i).wait()
        best, bidx = ln_block(i, best, bidx)
        r0 = pl.multiple_of(i * TM, TM)
        xn = xn_v[pl.ds(r0, TM), :]
        k = jnp.dot(xn, wk_v[...], preferred_element_type=F32)
        pk = _phi(k)
        z = z + jnp.sum(pk, axis=0, keepdims=True)
        pp = lax.dot_general(pk.astype(BF16), xn, (((0,), (0,)), ((), ())),
                             preferred_element_type=F32)
        p_v[...] += pp
        return best, bidx, z

    p_v[...] = jnp.zeros_like(p_v)
    best0 = jnp.full((TM, 1), -jnp.inf, F32)
    bidx0 = jnp.zeros((TM, 1), jnp.int32)
    z0 = jnp.zeros((1, D), F32)
    best, bidx, z = lax.fori_loop(0, NB, p1_body, (best0, bidx0, z0))

    gmax = jnp.max(best, axis=0, keepdims=True)
    idx = jnp.min(jnp.where(best == gmax, bidx, S - 1), axis=0, keepdims=True)
    idx_s = idx[0, 0]
    base = pl.multiple_of(jnp.clip((idx_s // 16) * 16, 0, S - 16), 16)

    wv_c.wait()
    wo_c.wait()
    ri = lax.broadcasted_iota(jnp.int32, (128, 128), 0) // Dh
    ci = lax.broadcasted_iota(jnp.int32, (128, 128), 1) // Dh
    blk = ri == ci
    for g in range(NG):
        gs = slice(g * 128, (g + 1) * 128)
        pg = p_v[gs, :].astype(BF16)
        kvg = jnp.dot(pg, wv_v[:, gs], preferred_element_type=F32)
        kvg = jnp.where(blk, kvg, 0.0).astype(BF16)
        m_v[gs, :] = jnp.dot(kvg, wo_v[gs, :], preferred_element_type=F32).astype(BF16)
        zg = jnp.broadcast_to(z[:, gs], (128, 128)).T
        zb_v[gs, :] = jnp.where(blk, zg, 0.0).astype(BF16)

    wg_c.wait()
    wu_c.wait()
    xs = xn_v[pl.ds(base, 16), :]
    g_ = jnp.dot(xs, wg_v[...], preferred_element_type=F32)
    u_ = jnp.dot(xs, wu_v[...], preferred_element_type=F32)
    h_ = (g_ * jax.nn.sigmoid(g_) * u_).astype(BF16)
    wd_c.wait()
    y16 = jnp.dot(h_, wd_v[...], preferred_element_type=F32)
    rows16 = lax.broadcasted_iota(jnp.int32, (16, 1), 0) + base
    y = jnp.sum(jnp.where(rows16 == idx, y16, 0.0), axis=0, keepdims=True)
    y = y * jax.nn.sigmoid(gmax)

    wq_c.wait()

    def p2_body(i, carry):
        r0 = pl.multiple_of(i * TM, TM)
        xn = xn_v[pl.ds(r0, TM), :]
        q = jnp.dot(xn, wq_v[...], preferred_element_type=F32)
        pq = _phi(q)
        pqb = pq.astype(BF16)
        dens = [jnp.dot(pqb[:, g * 128:(g + 1) * 128], zb_v[g * 128:(g + 1) * 128, :],
                        preferred_element_type=F32) for g in range(NG)]
        den = jnp.concatenate(dens, axis=-1) + PHI_EPS
        a = (pq / den).astype(BF16)
        att = jnp.dot(a, m_v[...], preferred_element_type=F32)
        rows = lax.broadcasted_iota(jnp.int32, (TM, 1), 0) + r0
        out = x_v[pl.ds(r0, TM), :].astype(F32) + xn.astype(F32) + att
        out = out + jnp.where(rows == idx, y, 0.0)
        o_v[pl.ds(r0, TM), :] = out.astype(BF16)
        o_copy(i).start()
        return carry

    lax.fori_loop(0, NB, p2_body, 0)
    for i in range(NB):
        o_copy(i).wait()


@jax.jit
def pallas_parallel_sum__linear_attn_block__moe_arch_mod__prompt_kernel(
    A_x: jax.Array,
    A_wqkv: jax.Array,
    A_wo: jax.Array,
    B_x: jax.Array,
    B_w_r: jax.Array,
    B_w_gate: jax.Array,
    B_w_up: jax.Array,
    B_w_down: jax.Array,
):
    del B_x
    B, S, D = A_x.shape
    F = B_w_gate.shape[1]
    assert B == 1
    NB = S // TM
    x2 = A_x.reshape(S, D)
    wr2 = B_w_r.reshape(1, D)

    any_spec = pl.BlockSpec(memory_space=pl.ANY)
    out = pl.pallas_call(
        functools.partial(_fused_kernel, S=S, D=D, F=F),
        out_shape=jax.ShapeDtypeStruct((S, D), BF16),
        in_specs=[any_spec, any_spec, any_spec,
                  pl.BlockSpec(memory_space=pltpu.VMEM),
                  any_spec, any_spec, any_spec],
        out_specs=any_spec,
        scratch_shapes=[
            pltpu.VMEM((S, D), BF16),
            pltpu.VMEM((S, D), BF16),
            pltpu.VMEM((D, D), BF16),
            pltpu.VMEM((D, D), BF16),
            pltpu.VMEM((D, D), BF16),
            pltpu.VMEM((D, D), BF16),
            pltpu.VMEM((D, F), BF16),
            pltpu.VMEM((D, F), BF16),
            pltpu.VMEM((F, D), BF16),
            pltpu.VMEM((D, D), F32),
            pltpu.VMEM((D, D), BF16),
            pltpu.VMEM((D, 128), BF16),
            pltpu.VMEM((S, D), BF16),
            pltpu.SemaphoreType.DMA((NB,)),
            pltpu.SemaphoreType.DMA((7,)),
            pltpu.SemaphoreType.DMA((NB,)),
        ],
        compiler_params=pltpu.CompilerParams(vmem_limit_bytes=100 * 1024 * 1024),
    )(x2, A_wqkv, A_wo, wr2, B_w_gate, B_w_up, B_w_down)
    return out.reshape(B, S, D)
```

```python
import contextlib
import functools

import jax
import jax.numpy as jnp
from jax import lax
import jax.experimental.pallas as pl
import jax.experimental.pallas.tpu as pltpu

F32 = jnp.float32
BF16 = jnp.bfloat16
U32 = jnp.uint32

H = 32
LN_EPS = 1e-5
PHI_EPS = 1e-6
NT_DIMS = (((1,), (1,)), ((), ()))
TN_DIMS = (((0,), (0,)), ((), ()))


def _phi(t):
    return jnp.where(t > 0, t + 1.0, jnp.exp(t)) + PHI_EPS


def _rnd(t):
    return t.astype(BF16).astype(F32)


def _pk(t):
    return pltpu.bitcast(t, U32)


def _upk(t):
    return pltpu.bitcast(t, BF16)


def _spread(main, side, first=0):
    out = []
    n, m = len(main), len(side)
    k = 0
    for j, it in enumerate(main):
        out.append(it)
        if j >= first:
            tgt = m * (j - first + 1) // (n - first)
            while k < tgt:
                out.append(side[k])
                k += 1
    return out


def _fused_kernel(x_hbm, wqkv_hbm, wo_hbm, wr_ref, wg_hbm, wu_hbm, wd_hbm, o_hbm,
                  x_v, xn_v, wq_v, wk_v, wv_v, wo_v, wg_v, wu_v, wd_v,
                  p_v, m_v, o_v, pk_v, a_v, wqt_v, zc_v, xb_v, hb_v,
                  fix_v, xsem, ksem, wsem, osem, zsem, fsem, *, S, D, F, TM, LNR, cfg):
    NB = S // TM
    Dh = D // H
    NG = D // 128
    HM = TM // 2
    zero = pl.semaphore_read(zsem)

    def scope(name):
        return jax.named_scope(name) if cfg.get('scopes') else contextlib.nullcontext()

    def x_copy(i):
        return pltpu.make_async_copy(
            x_hbm.at[pl.ds(i * TM, TM), :], x_v.at[pl.ds(i * TM, TM), :], xsem.at[i])

    def o_copy(i):
        return pltpu.make_async_copy(
            o_v.at[pl.ds(i * TM, TM), :], o_hbm.at[pl.ds(i * TM, TM), :], osem.at[i])

    def wk_copy(g):
        off = g * 128 if isinstance(g, int) else pl.multiple_of(g * 128, 128)
        return pltpu.make_async_copy(
            wqkv_hbm.at[:, pl.ds(D + off, 128)], wk_v.at[:, pl.ds(off, 128)], ksem.at[g])

    wq_c = pltpu.make_async_copy(wqkv_hbm.at[:, pl.ds(0, D)], wq_v, wsem.at[0])
    wv_c = pltpu.make_async_copy(wqkv_hbm.at[:, pl.ds(2 * D, D)], wv_v, wsem.at[1])
    wo_c = pltpu.make_async_copy(wo_hbm, wo_v, wsem.at[2])
    wg_c = pltpu.make_async_copy(wg_hbm, wg_v, wsem.at[3])
    wu_c = pltpu.make_async_copy(wu_hbm, wu_v, wsem.at[4])
    wd_c = pltpu.make_async_copy(wd_hbm, wd_v, wsem.at[5])

    x1_at = cfg.get('x1_at', 1)

    def wk_start_range(lo, hi):
        def body(g, c):
            wk_copy(g).start()
            return c
        if hi > lo:
            lax.fori_loop(lo, hi, body, 0)

    x_copy(0).start()
    wk_start_range(0, min(x1_at + 1, NG))
    if x1_at < NG:
        x_copy(1).start()
        wk_start_range(x1_at + 1, NG)

    def issue_rest():
        if x1_at >= NG:
            x_copy(1).start()
        for i in range(2, NB):
            x_copy(i).start()
        wq_c.start()
        wv_c.start()
        wo_c.start()
        wg_c.start()
        wu_c.start()
        wd_c.start()

    wr8 = wr_ref[...].astype(F32)
    wr = jnp.concatenate([wr8[j:j + 1, :] for j in range(NG)], axis=-1)

    st = {}
    st['best'] = jnp.full((LNR, 1), -jnp.inf, F32)
    st['bidx'] = jnp.zeros((LNR, 1), jnp.int32)
    st['z'] = [jnp.zeros((8, 128), F32) for _ in range(NG)]

    def rows(i):
        return slice(i * TM, (i + 1) * TM)

    def prow(i):
        return slice(i * HM, (i + 1) * HM)

    def cols(g, w=128):
        return slice(g * w, (g + 1) * w)

    def L(i, c):
        def f():
            if c == 0:
                xg = cfg.get('xgroups')
                if xg is None:
                    x_copy(i).wait()
                else:
                    for j in xg.get(i, ()):
                        x_copy(j).wait()
            r0 = i * TM + c * LNR
            x = x_v[r0:r0 + LNR, :].astype(F32)
            m = jnp.mean(x, axis=-1, keepdims=True)
            xc = x - m
            v = jnp.mean(xc * xc, axis=-1, keepdims=True)
            inv = 1.0 / _rnd(jnp.sqrt(_rnd(_rnd(v) + LN_EPS)))
            xn_v[r0 // 2:(r0 + LNR) // 2, :] = _pk((xc * inv).astype(BF16))
            r = jnp.sum(xc * wr, axis=-1, keepdims=True) * inv
            rr = lax.broadcasted_iota(jnp.int32, (LNR, 1), 0) + r0
            upd = r > st['best']
            st['best'] = jnp.where(upd, r, st['best'])
            st['bidx'] = jnp.where(upd, rr, st['bidx'])
        return f

    def K(i, g):
        def f():
            if i == 0:
                wk_copy(g).wait()
            st['k', i, g] = jnp.dot(_upk(xn_v[prow(i), :]), wk_v[:, cols(g)],
                                    preferred_element_type=F32)
        return f

    pkmode = cfg.get('pkmode', 0)

    def Fk(i, g):
        def f():
            pk = _phi(st.pop(('k', i, g)))
            acc = st['z'][g]
            for r in range(TM // 8):
                acc = acc + pk[r * 8:(r + 1) * 8, :]
            st['z'][g] = acc
            if pkmode == 0:
                pk_v[i % 2, cols(g), :] = pk.T.astype(BF16)
            elif pkmode == 1:
                pk_v[i % 2, :, cols(g)] = pk.astype(BF16)
        return f

    PC = cfg.get('PC', 256)
    PR = cfg.get('PR', 1024)

    def Pm(i, c, r):
        def f():
            cs = cols(c, PC)
            rs = slice(r * PR, (r + 1) * PR)
            rhs = _upk(xn_v[prow(i), cs])
            if pkmode == 0:
                pp = jnp.dot(pk_v[i % 2, rs, :], rhs, preferred_element_type=F32)
            else:
                pp = lax.dot_general(pk_v[i % 2, :, rs], rhs, TN_DIMS, preferred_element_type=F32)
            if i == 0:
                p_v[rs, cs] = pp
            else:
                p_v[rs, cs] += pp
        return f

    def WT(ft, kt):
        def f():
            if ft == 0 and kt == 0:
                wq_c.wait()
            t = wq_v[cols(kt), cols(ft)]
            wqt_v[pl.ds(pl.multiple_of(ft * 64 + zero, 64), 64), cols(kt)] = _pk(t.T)
        return f

    CW = cfg.get('CW', 512)
    RK = cfg.get('RK', 128)

    def SEL():
        def f():
            best, bidx = st['best'], st['bidx']
            gmax = jnp.max(best, axis=0, keepdims=True)
            idx = jnp.min(jnp.where(best == gmax, bidx, S - 1), axis=0, keepdims=True)
            st['gmax'], st['idx'] = gmax, idx
            base = jnp.clip((idx[0, 0] // 16) * 16, 0, S - 16)
            xs = _upk(xn_v[pl.ds(pl.multiple_of(base // 2, 8), 8), :]).astype(F32)
            rows16 = lax.broadcasted_iota(jnp.int32, (16, 1), 0) + base
            st['xsel'] = jnp.sum(jnp.where(rows16 == idx, xs, 0.0), axis=0, keepdims=True)
        return f

    def XB(g):
        def f():
            xb_v[cols(g), :] = jnp.broadcast_to(st['xsel'][:, cols(g)], (128, 128)).T
        return f

    def mv_item(key, w_v, tab_v, c, k0, nk, first):
        def f():
            acc = None if first else st.pop(key)
            TG = cfg.get('TG', 4)
            for r0 in range(0, nk // 8, TG):
                terms = []
                for r in range(r0, r0 + TG):
                    w = w_v[k0 + r * 8:k0 + (r + 1) * 8, cols(c, CW)].astype(F32)
                    xr = tab_v[k0 + r * 8:k0 + (r + 1) * 8, :]
                    xr = jnp.concatenate([xr] * (CW // 128), axis=-1)
                    terms.append(w * xr)
                while len(terms) > 1:
                    terms = [terms[j] + terms[j + 1] for j in range(0, len(terms), 2)]
                acc = terms[0] if acc is None else acc + terms[0]
            st[key] = acc
            dl = cfg.get('tie', 0)
            if dl:
                tv = acc[:, 0:128]
                for j in range(1, CW // 128):
                    tv = tv + acc[:, j * 128:(j + 1) * 128]
                st.setdefault(('tie', st['cur'] + dl), []).append(tv)
        return f

    def tie_u32(raw):
        ties = st.pop(('tie', st['cur']), None)
        if not ties:
            return raw
        t = ties[0]
        for u in ties[1:]:
            t = t + u
        tile = jnp.where(zero != 0, lax.bitcast_convert_type(t, U32), raw[0:8, 0:128])
        top = jnp.concatenate([tile, raw[0:8, 128:]], axis=1)
        return jnp.concatenate([top, raw[8:, :]], axis=0)

    def HC(c):
        def f():
            g_ = jnp.sum(st.pop(('g', c)), axis=0, keepdims=True)
            u_ = jnp.sum(st.pop(('u', c)), axis=0, keepdims=True)
            h_ = g_ * jax.nn.sigmoid(g_) * u_
            for j in range(CW // 128):
                f0 = c * CW + j * 128
                hbt = jnp.broadcast_to(h_[:, cols(j)], (128, 128)).T
                hb_v[f0:f0 + 128, :] = hbt
            if cfg.get('tie', 0):
                st.setdefault(('tie', st['cur'] + cfg['tie']), []).append(hbt[0:8, :])
        return f

    def YFIN():
        def f():
            ys = [jnp.sum(st.pop(('y', c)), axis=0, keepdims=True) for c in range(D // CW)]
            st['y'] = jnp.concatenate(ys, axis=-1) * jax.nn.sigmoid(st['gmax'])
        return f

    def wait_item(cp):
        def f():
            cp.wait()
        return f

    moe_gu = [SEL()] + [XB(g) for g in range(NG)] + [wait_item(wg_c), wait_item(wu_c)]
    for c in range(F // CW):
        for key, w_v in ((('g', c), wg_v), (('u', c), wu_v)):
            for k0 in range(0, D, RK):
                moe_gu.append(mv_item(key, w_v, xb_v, c, k0, RK, k0 == 0))
        moe_gu.append(HC(c))
    moe_d = [wait_item(wd_c)]
    for c in range(D // CW):
        for k0 in range(0, F, RK):
            moe_d.append(mv_item(('y', c), wd_v, hb_v, c, k0, RK, k0 == 0))
    moe_d.append(YFIN())
    moe = moe_gu + moe_d
    if cfg.get('nomoe'):
        def y0():
            st['y'] = st['xsel']
        moe = [SEL(), y0, wait_item(wg_c), wait_item(wu_c), wait_item(wd_c)]

    ri = lax.broadcasted_iota(jnp.int32, (128, 128), 0) // Dh
    ci = lax.broadcasted_iota(jnp.int32, (128, 128), 1) // Dh
    blk = ri == ci

    def ZT(g):
        def f():
            zrow = jnp.sum(st['z'][g], axis=0, keepdims=True)
            zc_v[cols(g), :] = jnp.broadcast_to(zrow, (128, 128)).T
        return f

    def KV(g):
        def f():
            if g == 0:
                wv_c.wait()
            pg = p_v[cols(g), :].astype(BF16)
            kvg = jnp.dot(pg, wv_v[:, cols(g)], preferred_element_type=F32)
            st['kv', g] = jnp.where(blk, kvg, 0.0).astype(BF16)
        return f

    def MM(g):
        def f():
            if g == 0:
                wo_c.wait()
            m_v[cols(g), :] = jnp.dot(st.pop(('kv', g)), wo_v[cols(g), :],
                                      preferred_element_type=F32).astype(BF16)
        return f

    QC = cfg.get('QC', 256)
    NQ = D // QC
    NT = S // 128

    KS = cfg.get('KS', 1)
    KW = D // KS

    def QT(t, c, ks):
        def f():
            kc = slice(ks * KW, (ks + 1) * KW)
            lhs = _upk(tie_u32(wqt_v[c * QC // 2:(c + 1) * QC // 2, kc]))
            rhs = _upk(xn_v[t * 64:(t + 1) * 64, kc])
            r = lax.dot_general(lhs, rhs, NT_DIMS, preferred_element_type=F32)
            st['q', t, c] = r if ks == 0 else st['q', t, c] + r
        return f

    GS = cfg.get('GS', 1)

    def G(t, c, gs):
        def f():
            nh = QC // Dh // GS
            q = st['q', t, c]
            if gs == GS - 1:
                st.pop(('q', t, c))
            outs = []
            for h in range(gs * nh, (gs + 1) * nh):
                f0 = h * Dh
                ph = _phi(q[f0:f0 + Dh, :])
                zc = zc_v[c * QC + f0:c * QC + f0 + Dh, :]
                t_ = ph * zc
                s = (t_[0:8] + t_[8:16]) + (t_[16:24] + t_[24:32])
                den = jnp.sum(s, axis=0, keepdims=True) + PHI_EPS
                outs.append(ph * (1.0 / den))
            a = jnp.concatenate(outs, axis=0)
            c0 = c * QC + gs * nh * Dh
            a_v[t * 64:(t + 1) * 64, c0:c0 + nh * Dh] = _pk(a.T.astype(BF16))
        return f

    EW = cfg.get('EW', 128)
    NE = D // EW
    ES = cfg.get('ES', 1)

    def O(i, g, ks):
        def f():
            kc = slice(ks * KW, (ks + 1) * KW)
            r = jnp.dot(_upk(tie_u32(a_v[prow(i), kc])), m_v[kc, cols(g, EW)],
                        preferred_element_type=F32)
            st['att', i, g] = r if ks == 0 else st['att', i, g] + r
        return f

    def E(i, g, es):
        def f():
            att = st['att', i, g]
            if es == ES - 1:
                st.pop(('att', i, g))
            cs = cols(g, EW)
            RW = TM // ES
            r0 = i * TM + es * RW
            att = att[es * RW:(es + 1) * RW, :]
            rr = lax.broadcasted_iota(jnp.int32, (RW, 1), 0) + r0
            out = (x_v[r0:r0 + RW, cs].astype(F32)
                   + _upk(xn_v[r0 // 2:(r0 + RW) // 2, cs]).astype(F32) + att)
            if i == NB - 1:
                out = out + jnp.where(rr == st['idx'], st['y'][:, cs], 0.0)
            o_v[r0:r0 + RW, cs] = out.astype(BF16)
            if g == NE - 1 and es == ES - 1:
                o_copy(i).start()
        return f

    NLC = TM // LNR
    plan = []
    pro = [L(0, c) for c in range(NLC)]

    lq = [L(1, c) for c in range(NLC)]
    l1_from = cfg.get('l1_from', 3)
    for g in range(NG):
        it = [K(0, g)]
        if g == cfg.get('rest_at', 5):
            it.append(issue_rest)
        if g > 0:
            it.append(Fk(0, g - 1))
        if g >= l1_from:
            ng = NG - l1_from
            n = NLC * (g - l1_from + 1) // ng - NLC * (g - l1_from) // ng
            for _ in range(n):
                it.append(lq.pop(0))
        plan.append((0, it))
    pend = [Fk(0, NG - 1)]
    wt_items = [WT(ft, kt) for ft in range(NG) for kt in range(NG)]
    wt_blocks = cfg.get('wt_blocks', (2, 3, 4, 5))
    PW = (PC // 128) * (PR // 128) * 128 / 512.0 / 4
    PW = PC * PR * TM / (128.0 * 1024 * 256)
    moe_from_blk = cfg.get('moe_from', NB - 2)
    for i in range(NB):
        wgt = 1.0 if i >= moe_from_blk else 0.0
        pitems = [Pm(i, c, r) for c in range(D // PC) for r in range(D // PR)]
        if i + 1 < NB:
            plan.append((wgt, [K(i + 1, 0)] + pend))
            pend = []
            side = [Fk(i + 1, 0)]
            if i + 2 < NB:
                side += [L(i + 2, c) for c in range(NLC)]
            ns_, np_ = len(side), len(pitems)
            for j, it in enumerate(pitems):
                n = ns_ * (j + 1) // np_ - ns_ * j // np_
                plan.append((wgt * PW * (0.5 if side else 1.0), [it] + [side.pop(0) for _ in range(n)]))
            for g in range(1, NG):
                it = [K(i + 1, g)]
                if g > 1:
                    it.append(Fk(i + 1, g - 1))
                if i in wt_blocks:
                    tot = 64 // len(wt_blocks)
                    n = tot * g // (NG - 1) - tot * (g - 1) // (NG - 1)
                    for _ in range(n):
                        it.append(wt_items.pop(0))
                plan.append((wgt, it))
            pend = [Fk(i + 1, NG - 1)]
        else:
            plan.append((wgt, [QT(0, 0, ks) for ks in range(KS)] + pend))
            pend = []
            for j, it in enumerate(pitems):
                plan.append((wgt * PW, [it]))
    assert not wt_items
    n_p1 = len(plan)

    pend = [ZT(g) for g in range(NG)] + [G(0, 0, gs) for gs in range(GS)]
    qitems = [(t, c) for t in range(NT) for c in range(NQ)][1:]
    n_pre = cfg.get('n_pre', 3)
    wq_ = cfg.get('w_q', 1.0)
    wo_ = cfg.get('w_o', 1.0)

    def emit(mains, wgt, after):
        nonlocal pend
        n = len(mains)
        m_ = len(pend)
        for j, mn in enumerate(mains):
            share = pend[m_ * j // n:m_ * (j + 1) // n]
            plan.append((wgt / n, [mn] + share))
        pend = list(after)

    def emit_q(tc):
        emit([QT(tc[0], tc[1], ks) for ks in range(KS)], wq_, [G(tc[0], tc[1], gs) for gs in range(GS)])

    for tc in qitems[:n_pre]:
        emit_q(tc)
    kvm = [KV(0)]
    for g in range(NG):
        if g + 1 < NG:
            kvm.append(KV(g + 1))
        kvm.append(MM(g))
    for it in kvm:
        emit([it], cfg.get('w_kvm', 0.5), [])
    rest = qitems[n_pre:]
    oitems = [(i, g) for i in range(NB) for g in range(NE)]
    qdone = n_pre + 1
    lead = cfg.get('lead', (TM // 128) * NQ + 1)
    y_deadline = None
    for n, (i, g) in enumerate(oitems):
        while rest and qdone < lead + n * (NQ * (TM // 128)) // NE:
            emit_q(rest.pop(0))
            qdone += 1
        assert (not rest) or qdone >= (i + 1) * (TM // 128) * NQ + 1
        if i == NB - 1 and g == 0:
            y_deadline = len(plan)
        emit([O(i, g, ks) for ks in range(KS)], wo_ * EW / 128.0, [E(i, g, es) for es in range(ES)])
    assert not rest
    plan.append((0, pend))

    tot_w = sum(w for w, _ in plan[:y_deadline])
    acc_w = 0.0
    k = 0
    for j in range(y_deadline):
        w, items = plan[j]
        acc_w += w
        tgt = int(round(len(moe) * acc_w / tot_w))
        pos = cfg.get('moe_pos', 0)
        while k < tgt:
            if pos == 0:
                items.append(moe[k])
            else:
                items.insert(min(1, len(items)), moe[k])
            k += 1
    assert k == len(moe)

    with scope('prologue'):
        for f in pro:
            f()
    with scope('phase1'):
        for j, (_, items) in enumerate(plan[:n_p1]):
            st['cur'] = j
            for f in items:
                f()
    with scope('phase2'):
        for j, (_, items) in enumerate(plan[n_p1:]):
            st['cur'] = n_p1 + j
            for f in items:
                f()
    with scope('tail'):
        for i in range(NB - 1):
            o_copy(i).wait()
        idx, y = st['idx'], st['y']
        idx_s = idx[0, 0]
        base = jnp.where(idx_s < (NB - 1) * TM, (idx_s // 16) * 16, 0)
        base = pl.multiple_of(jnp.clip(base, 0, S - 16), 16)
        o16 = o_v[pl.ds(base, 16), :].astype(F32)
        rows16 = lax.broadcasted_iota(jnp.int32, (16, 1), 0) + base
        fix_v[...] = (o16 + jnp.where(rows16 == idx, y, 0.0)).astype(BF16)
        fix_c = pltpu.make_async_copy(fix_v, o_hbm.at[pl.ds(base, 16), :], fsem)
        fix_c.start()
        o_copy(NB - 1).wait()
        fix_c.wait()


def make(TM=256, LNR=32, **cfg):
    @jax.jit
    def kern(A_x, A_wqkv, A_wo, B_x, B_w_r, B_w_gate, B_w_up, B_w_down):
        del B_x
        B, S, D = A_x.shape
        F = B_w_gate.shape[1]
        assert B == 1
        NB = S // TM
        x2 = A_x.reshape(S, D)
        wr2 = B_w_r.reshape(D // 128, 128)

        any_spec = pl.BlockSpec(memory_space=pl.ANY)
        cp = dict(vmem_limit_bytes=110 * 1024 * 1024)
        if cfg.get('flags'):
            cp['flags'] = cfg['flags']
        pkshape = (2, D, TM) if cfg.get('pkmode', 0) == 0 else (2, TM, D)
        out = pl.pallas_call(
            functools.partial(_fused_kernel, S=S, D=D, F=F, TM=TM, LNR=LNR, cfg=cfg),
            out_shape=jax.ShapeDtypeStruct((S, D), BF16),
            in_specs=[any_spec, any_spec, any_spec,
                      pl.BlockSpec(memory_space=pltpu.VMEM),
                      any_spec, any_spec, any_spec],
            out_specs=any_spec,
            scratch_shapes=[
                pltpu.VMEM((S, D), BF16),
                pltpu.VMEM((S // 2, D), U32),
                pltpu.VMEM((D, D), BF16),
                pltpu.VMEM((D, D), BF16),
                pltpu.VMEM((D, D), BF16),
                pltpu.VMEM((D, D), BF16),
                pltpu.VMEM((D, F), BF16),
                pltpu.VMEM((D, F), BF16),
                pltpu.VMEM((F, D), BF16),
                pltpu.VMEM((D, D), F32),
                pltpu.VMEM((D, D), BF16),
                pltpu.VMEM((S, D), BF16),
                pltpu.VMEM(pkshape, BF16),
                pltpu.VMEM((S // 2, D), U32),
                pltpu.VMEM((D // 2, D), U32),
                pltpu.VMEM((D, 128), F32),
                pltpu.VMEM((D, 128), F32),
                pltpu.VMEM((F, 128), F32),
                pltpu.VMEM((16, D), BF16),
                pltpu.SemaphoreType.DMA((NB,)),
                pltpu.SemaphoreType.DMA((8,)),
                pltpu.SemaphoreType.DMA((6,)),
                pltpu.SemaphoreType.DMA((NB,)),
                pltpu.SemaphoreType.REGULAR,
                pltpu.SemaphoreType.DMA,
            ],
            compiler_params=pltpu.CompilerParams(**cp),
        )(x2, A_wqkv, A_wo, wr2, B_w_gate, B_w_up, B_w_down)
        return out.reshape(B, S, D)
    return kern


pallas_parallel_sum__linear_attn_block__moe_arch_mod__prompt_kernel = make(
    TG=1, moe_from=8, tie=4, RK=256)
```

```python
import contextlib
import functools

import jax
import jax.numpy as jnp
from jax import lax
import jax.experimental.pallas as pl
import jax.experimental.pallas.tpu as pltpu

F32 = jnp.float32
BF16 = jnp.bfloat16
U32 = jnp.uint32

H = 32
LN_EPS = 1e-5
PHI_EPS = 1e-6
NT_DIMS = (((1,), (1,)), ((), ()))


def _phi(t):
    return jnp.where(t > 0, t + 1.0, jnp.exp(t)) + PHI_EPS


def _rnd(t):
    return t.astype(BF16).astype(F32)


def _pk(t):
    return pltpu.bitcast(t, U32)


def _upk(t):
    return pltpu.bitcast(t, BF16)


ST_A = (((0, 1), (3, 1)), ((2, 1), (3, 1)), ((0, 1),), ((3, 1),),
        ((0, 1), (1, 1)), ((2, 1), (0, -1)), ((1, 1), (3, -1)))
ST_B = (((0, 1), (3, 1)), ((0, 1),), ((1, 1), (3, -1)), ((2, 1), (0, -1)),
        ((3, 1),), ((0, 1), (1, 1)), ((2, 1), (3, 1)))
ST_C = (((0, 1), (3, 1)), ((2, 1), (3, -1)), ((1, 1), (3, 1)), ((0, 1), (2, 1)),
        ((0, -1), (1, 1)), ((3, 1),), ((0, 1),))
ST_LAST = {}
for _m, _cs in enumerate(ST_C):
    for _c, _ in _cs:
        ST_LAST[_c] = _m


def _comb(blocks, terms):
    out = None
    for b, sg in terms:
        v = blocks[b]
        if out is None:
            out = v if sg > 0 else -v
        else:
            out = out + v if sg > 0 else out - v
    return out


def _fused_kernel(x_hbm, wqkv_hbm, wo_hbm, wr_hbm, wg_hbm, wu_hbm, wd_hbm, o_hbm,
                  x_v, xn_v, wq_v, wk_v, wvo_v, wgu_v, wd_v,
                  p_v, m7_v, o_v, pk_v, a7_v, wqt_v, zc_v, xb_v, hb_v, xs_v, wk7_v,
                  fix_v, wr_ref, xsem, ksem, wsem, osem, fsem, rsem, *, S, D, F, TM, LNR, cfg):
    NB = S // TM
    Dh = D // H
    NG = D // 128
    HM = TM // 2
    HD = D // 2
    TH = TM // 2
    PH = TH // 2
    wv_v, wo_v = wvo_v.at[0], wvo_v.at[1]
    wg_v, wu_v = wgu_v.at[0], wgu_v.at[1]
    SQ = cfg.get('SQ', 1)
    SO = cfg.get('SO', 1)
    SK = cfg.get('SK', 0)
    need_xs = SQ or SK < NB

    def scope(name):
        return jax.named_scope(name) if cfg.get('scopes') else contextlib.nullcontext()

    XG = cfg.get('XG', ((0, 1), (1, 2), (2, 4), (4, 8)))

    def x_copy(j):
        lo, hi = XG[j]
        return pltpu.make_async_copy(
            x_hbm.at[pl.ds(lo * TM, (hi - lo) * TM), :], x_v.at[pl.ds(lo * TM, (hi - lo) * TM), :],
            xsem.at[j])

    def o_copy(i):
        return pltpu.make_async_copy(
            o_v.at[pl.ds(i * TM, TM), :], o_hbm.at[pl.ds(i * TM, TM), :], osem.at[0])

    def ol_copy(j):
        return pltpu.make_async_copy(
            o_v.at[pl.ds((NB - 1) * TM, TM), pl.ds(j * 128, 128)],
            o_hbm.at[pl.ds((NB - 1) * TM, TM), pl.ds(j * 128, 128)], osem.at[1])

    KPL = cfg.get('KPL', (256, 256, 256, 256))
    KOFF = [sum(KPL[:j]) for j in range(len(KPL))]
    NP = len(KPL)

    def wk_copy(j):
        return pltpu.make_async_copy(
            wqkv_hbm.at[:, pl.ds(D + KOFF[j], KPL[j])], wk_v.at[:, pl.ds(KOFF[j], KPL[j])], ksem.at[j])

    wq_c = pltpu.make_async_copy(wqkv_hbm.at[:, pl.ds(0, D)], wq_v, wsem.at[0])
    wv_c = pltpu.make_async_copy(wqkv_hbm.at[:, pl.ds(2 * D, D)], wv_v, wsem.at[1])
    wo_c = pltpu.make_async_copy(wo_hbm, wo_v, wsem.at[1])
    wvo_w = pltpu.make_async_copy(wvo_v, wvo_v, wsem.at[1])
    wg_c = pltpu.make_async_copy(wg_hbm, wg_v, wsem.at[2])
    wu_c = pltpu.make_async_copy(wu_hbm, wu_v, wsem.at[2])
    wgu_w = pltpu.make_async_copy(wgu_v, wgu_v, wsem.at[2])
    wd_c = pltpu.make_async_copy(wd_hbm, wd_v, wsem.at[3])
    wr_c = pltpu.make_async_copy(wr_hbm, wr_ref, rsem)
    first = [wr_c, x_copy(0)] + [wk_copy(j) for j in range(NP)] + [x_copy(1)]

    def start_in_order(cps):
        def body(k, c):
            for j, cp in enumerate(cps):
                pl.when(k == j)(cp.start)
            return c
        lax.fori_loop(0, len(cps), body, 0)

    start_in_order(first)

    issue_at = cfg.get('issue_at', {2: (2,), 4: (3,), 6: ('wq',), 8: ('w2',)})

    def issue(g):
        def f():
            for it in issue_at.get(g, ()):
                if it == 'wq':
                    wq_c.start()
                elif it == 'w2':
                    for cp in (wv_c, wo_c, wg_c, wu_c, wd_c):
                        cp.start()
                else:
                    x_copy(it).start()
        return f

    wr_c.wait()
    wr8 = wr_ref[...].astype(F32)
    zero = lax.shift_right_logical(
        lax.bitcast_convert_type(jnp.abs(wr8[0:1, 0:1]), jnp.int32), 31)[0, 0]
    wr = jnp.concatenate([wr8[j:j + 1, :] for j in range(NG)], axis=-1)

    st = {}
    st['best'] = jnp.full((LNR, 1), -jnp.inf, F32)
    st['bidx'] = jnp.zeros((LNR, 1), jnp.int32)
    st['z'] = [jnp.zeros((8, 128), F32) for _ in range(NG)]

    def rows(i):
        return slice(i * TM, (i + 1) * TM)

    def prow(i):
        return slice(i * HM, (i + 1) * HM)

    def cols(g, w=128):
        return slice(g * w, (g + 1) * w)

    XSUM = [m for m in range(7) if len(ST_A[m]) > 1]

    def xn_op(i, m):
        if len(ST_A[m]) == 1:
            b = ST_A[m][0][0]
            r0 = i * HM + (b // 2) * PH
            return xn_v[r0:r0 + PH, cols(b % 2, HD)]
        return xs_v[XSUM.index(m), i * PH:(i + 1) * PH, :]

    def L(i, c):
        def f():
            if c == 0:
                for j, (lo, hi) in enumerate(XG):
                    if lo == i:
                        x_copy(j).wait()
                if i == cfg.get('wq_at', 4):
                    wq_c.wait()
            r0 = i * TM + c * LNR
            x = x_v[r0:r0 + LNR, :].astype(F32)
            m = jnp.mean(x, axis=-1, keepdims=True)
            xc = x - m
            v = jnp.mean(xc * xc, axis=-1, keepdims=True)
            inv = 1.0 / _rnd(jnp.sqrt(_rnd(_rnd(v) + LN_EPS)))
            xn = xc * inv
            xn_v[r0 // 2:(r0 + LNR) // 2, :] = _pk(xn.astype(BF16))
            if need_xs and c * LNR >= TH:
                r1 = r0 - TH
                top = _upk(xn_v[r1 // 2:(r1 + LNR) // 2, :]).astype(F32)
                blk = (top[:, :HD], top[:, HD:], xn[:, :HD], xn[:, HD:])
                q0 = i * PH + (c * LNR - TH) // 2
                for k, mm in enumerate(XSUM):
                    xs_v[k, q0:q0 + LNR // 2, :] = _pk(_comb(blk, ST_A[mm]).astype(BF16))
            r = jnp.sum(xc * wr, axis=-1, keepdims=True) * inv
            rr = lax.broadcasted_iota(jnp.int32, (LNR, 1), 0) + r0
            upd = r > st['best']
            st['best'] = jnp.where(upd, r, st['best'])
            st['bidx'] = jnp.where(upd, rr, st['bidx'])
        return f

    def K(i, g):
        def f():
            if i == 0 and g * 128 in KOFF:
                wk_copy(KOFF.index(g * 128)).wait()
            st['k', i, g] = jnp.dot(_upk(xn_v[prow(i), :]), wk_v[:, cols(g)],
                                    preferred_element_type=F32)
        return f

    def acc_products(key, m, val):
        for c, sg in ST_C[m]:
            k = key + (c,)
            if k in st:
                st[k] = st[k] + val if sg > 0 else st[k] - val
            else:
                st[k] = val if sg > 0 else -val

    def wk_op(m, j):
        if len(ST_B[m]) == 1:
            b = ST_B[m][0][0]
            return wk_v[cols(b // 2, HD), cols((b % 2) * 4 + j)]
        return _upk(wk7_v[BSUM.index(m), :, cols(j)])

    BSUM = [m for m in range(7) if len(ST_B[m]) > 1]

    def KS7(i, j, m):
        def f():
            val = jnp.dot(_upk(xn_op(i, m)), wk_op(m, j), preferred_element_type=F32)
            acc_products(('kc', i, j), m, val)
            if m == 6:
                c = [st.pop(('kc', i, j, b)) for b in range(4)]
                st['k', i, j] = jnp.concatenate([c[0], c[2]], axis=0)
                st['k', i, 4 + j] = jnp.concatenate([c[1], c[3]], axis=0)
        return f

    def WK7(m, rc):
        def f():
            rs = 128
            blk = {}
            for b, _ in ST_B[m]:
                r0 = (b // 2) * HD + rc * rs
                blk[b] = wk_v[r0:r0 + rs, cols(b % 2, HD)].astype(F32)
            wk7_v[BSUM.index(m), rc * rs // 2:(rc + 1) * rs // 2, :] = _pk(_comb(blk, ST_B[m]).astype(BF16))
        return f

    def Fk(i, g):
        def f():
            pk = _phi(st.pop(('k', i, g)))
            acc = st['z'][g]
            for r in range(TM // 8):
                acc = acc + pk[r * 8:(r + 1) * 8, :]
            st['z'][g] = acc
            pk_v[i % 2, cols(g), :] = pk.T.astype(BF16)
        return f

    PC = cfg.get('PC', 512)
    PR = cfg.get('PR', 1024)

    def Pm(i, c, r):
        def f():
            cs = cols(c, PC)
            rs = slice(r * PR, (r + 1) * PR)
            rhs = _upk(xn_v[prow(i), cs])
            pp = jnp.dot(pk_v[i % 2, rs, :], rhs, preferred_element_type=F32)
            if i == 0:
                p_v[rs, cs] = pp
            else:
                p_v[rs, cs] += pp
        return f

    def WT(m, ft, kt):
        def f():
            if SQ:
                blk = {}
                for b, _ in ST_B[m]:
                    blk[b] = wq_v[cols((b // 2) * 4 + kt), cols((b % 2) * 4 + ft)].astype(F32)
                t = _comb(blk, ST_B[m]).T.astype(BF16)
                wqt_v[m, pl.ds(pl.multiple_of(ft * 64 + zero, 64), 64), cols(kt)] = _pk(t)
            else:
                t = wq_v[cols(kt), cols(ft)]
                wqt_v[kt // 4, pl.ds(pl.multiple_of(ft * 64 + zero, 64), 64), cols(kt % 4)] = _pk(t.T)
        return f

    CW = cfg.get('CW', 512)
    RK = cfg.get('RK', 256)

    def SEL():
        def f():
            best, bidx = st['best'], st['bidx']
            gmax = jnp.max(best, axis=0, keepdims=True)
            idx = jnp.min(jnp.where(best == gmax, bidx, S - 1), axis=0, keepdims=True)
            st['gmax'], st['idx'] = gmax, idx
            base = jnp.clip((idx[0, 0] // 16) * 16, 0, S - 16)
            xs = _upk(xn_v[pl.ds(pl.multiple_of(base // 2, 8), 8), :]).astype(F32)
            rows16 = lax.broadcasted_iota(jnp.int32, (16, 1), 0) + base
            st['xsel'] = jnp.sum(jnp.where(rows16 == idx, xs, 0.0), axis=0, keepdims=True)
        return f

    def XB(g):
        def f():
            xb_v[cols(g), :] = jnp.broadcast_to(st['xsel'][:, cols(g)], (128, 128)).T
        return f

    def mv_item(key, w_v, tab_v, c, k0, nk, first):
        def f():
            acc = None if first else st.pop(key)
            for r in range(nk // 8):
                w = w_v[k0 + r * 8:k0 + (r + 1) * 8, cols(c, CW)].astype(F32)
                xr = tab_v[k0 + r * 8:k0 + (r + 1) * 8, :]
                xr = jnp.concatenate([xr] * (CW // 128), axis=-1)
                acc = w * xr if acc is None else acc + w * xr
            st[key] = acc
            dl = cfg.get('tie', 4)
            if dl:
                tv = acc[:, 0:128]
                for j in range(1, CW // 128):
                    tv = tv + acc[:, j * 128:(j + 1) * 128]
                st.setdefault(('tie', st['cur'] + dl), []).append(tv)
        return f

    def tie_u32(raw):
        ties = st.pop(('tie', st['cur']), None)
        if not ties:
            return raw
        t = ties[0]
        for u in ties[1:]:
            t = t + u
        tile = jnp.where(zero != 0, lax.bitcast_convert_type(t, U32), raw[0:8, 0:128])
        top = jnp.concatenate([tile, raw[0:8, 128:]], axis=1)
        return jnp.concatenate([top, raw[8:, :]], axis=0)

    def HC(c):
        def f():
            g_ = jnp.sum(st.pop(('g', c)), axis=0, keepdims=True)
            u_ = jnp.sum(st.pop(('u', c)), axis=0, keepdims=True)
            h_ = g_ * jax.nn.sigmoid(g_) * u_
            for j in range(CW // 128):
                f0 = c * CW + j * 128
                hbt = jnp.broadcast_to(h_[:, cols(j)], (128, 128)).T
                hb_v[f0:f0 + 128, :] = hbt
            if cfg.get('tie', 4):
                st.setdefault(('tie', st['cur'] + cfg.get('tie', 4)), []).append(hbt[0:8, :])
        return f

    def YFIN():
        def f():
            ys = [jnp.sum(st.pop(('y', c)), axis=0, keepdims=True) for c in range(D // CW)]
            st['y'] = jnp.concatenate(ys, axis=-1) * jax.nn.sigmoid(st['gmax'])
        return f

    moe = [SEL()] + [XB(g) for g in range(NG)]
    for c in range(F // CW):
        for key, w_v in ((('g', c), wg_v), (('u', c), wu_v)):
            for k0 in range(0, D, RK):
                moe.append(mv_item(key, w_v, xb_v, c, k0, RK, k0 == 0))
        moe.append(HC(c))
    for c in range(D // CW):
        for k0 in range(0, F, RK):
            moe.append(mv_item(('y', c), wd_v, hb_v, c, k0, RK, k0 == 0))
    moe.append(YFIN())
    if cfg.get('nomoe'):
        def y0():
            st['y'] = st['xsel']
        moe = [SEL(), y0]

    ri = lax.broadcasted_iota(jnp.int32, (128, 128), 0) // Dh
    ci = lax.broadcasted_iota(jnp.int32, (128, 128), 1) // Dh
    blk_mask = ri == ci

    def ZT(g):
        def f():
            zrow = jnp.sum(st['z'][g], axis=0, keepdims=True)
            zc_v[cols(g), :] = jnp.broadcast_to(zrow, (128, 128)).T
        return f

    def KV(g):
        def f():
            if g == 0:
                wvo_w.wait()
                wgu_w.wait()
                wd_c.wait()
            pg = p_v[cols(g), :].astype(BF16)
            kvg = jnp.dot(pg, wv_v[:, cols(g)], preferred_element_type=F32)
            st['kv', g] = jnp.where(blk_mask, kvg, 0.0).astype(BF16)
        return f

    def MM(g):
        def f():
            mg = jnp.dot(st.pop(('kv', g)), wo_v[cols(g), :], preferred_element_type=F32)
            if not SO:
                m7_v[g // 4, (g % 4) * 64:(g % 4 + 1) * 64, :] = _pk(mg.astype(BF16))
                return
            st['m', g] = mg
            if g >= 4:
                top, bot = st.pop(('m', g - 4)), st.pop(('m', g))
                blk = (top[:, :HD], top[:, HD:], bot[:, :HD], bot[:, HD:])
                r = g - 4
                for m in range(7):
                    m7_v[m, r * 64:(r + 1) * 64, 0:HD] = _pk(_comb(blk, ST_B[m]).astype(BF16))
        return f

    QC = cfg.get('QC', 256)
    NQ = HD // QC

    def QT(i, c, m):
        def f():
            if SQ:
                lhs = _upk(tie_u32(wqt_v[m, c * QC // 2:(c + 1) * QC // 2, :]))
                val = lax.dot_general(lhs, _upk(xn_op(i, m)), NT_DIMS, preferred_element_type=F32)
                acc_products(('qc', i, c), m, val)
            else:
                fh, th = m % 2, m // 2
                f0 = fh * HD + c * QC
                lhs = jnp.concatenate(
                    [wqt_v[0, f0 // 2:(f0 + QC) // 2, :], wqt_v[1, f0 // 2:(f0 + QC) // 2, :]], axis=1)
                r0 = i * HM + th * PH
                st[('qc', i, c, m)] = lax.dot_general(
                    _upk(tie_u32(lhs)), _upk(xn_v[r0:r0 + PH, :]), NT_DIMS, preferred_element_type=F32)
        return f

    def GA(i, c, b):
        def f():
            q = st.pop(('qc', i, c, b))
            f00 = (b % 2) * HD + c * QC
            outs = []
            for h in range(QC // Dh):
                f0 = h * Dh
                ph = _phi(q[f0:f0 + Dh, :])
                zc = zc_v[f00 + f0:f00 + f0 + Dh, :]
                t_ = ph * zc
                s = (t_[0:8] + t_[8:16]) + (t_[16:24] + t_[24:32])
                den = jnp.sum(s, axis=0, keepdims=True) + PHI_EPS
                outs.append(ph * (1.0 / den))
            st[('a', i, c, b)] = jnp.concatenate(outs, axis=0)
        return f

    def GS(i, c, m):
        def f():
            blk = {b: st[('a', i, c, b)] for b in range(4)}
            if SO:
                val = _comb(blk, ST_A[m])
                a7_v[m, i * PH:(i + 1) * PH, cols(c, QC)] = _pk(val.T.astype(BF16))
                if m == 6:
                    for b in range(4):
                        st.pop(('a', i, c, b))
            else:
                th, fh = m // 2, m % 2
                a7_v[fh, i * HM + th * PH:i * HM + (th + 1) * PH, cols(c, QC)] = _pk(
                    st.pop(('a', i, c, m)).T.astype(BF16))
        return f

    def m_op(m, j):
        return _upk(m7_v[m, :, cols(j)])

    def O(i, j, m):
        def f():
            if SO:
                lhs = _upk(tie_u32(a7_v[m, i * PH:(i + 1) * PH, :]))
                val = jnp.dot(lhs, m_op(m, j), preferred_element_type=F32)
                acc_products(('oc', i, j), m, val)
            else:
                th, eh = m // 2, m % 2
                r0 = i * HM + th * PH
                lhs = jnp.concatenate([a7_v[0, r0:r0 + PH, :], a7_v[1, r0:r0 + PH, :]], axis=1)
                g = eh * 4 + j
                rhs = jnp.concatenate([m7_v[0, :, cols(g)], m7_v[1, :, cols(g)]], axis=0)
                st[('oc', i, j, m)] = jnp.dot(_upk(tie_u32(lhs)), _upk(rhs), preferred_element_type=F32)
        return f

    def E(i, j, b):
        def f():
            att = st.pop(('oc', i, j, b))
            th, eh = b // 2, b % 2
            cs = cols(eh * 4 + j)
            r0 = i * TM + th * TH
            rr = lax.broadcasted_iota(jnp.int32, (TH, 1), 0) + r0
            out = (x_v[r0:r0 + TH, cs].astype(F32)
                   + _upk(xn_v[r0 // 2:(r0 + TH) // 2, cs]).astype(F32) + att)
            if i == NB - 1:
                out = out + jnp.where(rr == st['idx'], st['y'][:, cs], 0.0)
            o_v[r0:r0 + TH, cs] = out.astype(BF16)
            done = st.setdefault(('edone', i), set())
            done.add((j, b))
            if i == NB - 1:
                if (j, eh) in done and (j, 2 + eh) in done:
                    ol_copy(eh * 4 + j).start()
            elif len(done) == 16:
                o_copy(i).start()
        return f

    NLC = TM // LNR
    plan = []
    pro = [L(0, c) for c in range(NLC)]

    def k_items(i):
        if i >= SK:
            out = []
            for j in range(4):
                for m in range(7):
                    out.append((KS7(i, j, m), [Fk(i, j), Fk(i, 4 + j)] if m == 6 else []))
            return out
        return [(K(i, g), [Fk(i, g)]) for g in range(NG)]

    def spread(mains, side):
        nonlocal pend
        n, m_ = len(mains), len(side)
        for j, (it, rel) in enumerate(mains):
            plan.append((0.0, [it] + pend + side[m_ * j // n:m_ * (j + 1) // n]))
            pend = list(rel)

    pend = []
    k0 = k_items(0)
    for g, (it, rel) in enumerate(k0):
        plan.append((0.0, [it, issue(g)] + pend))
        pend = list(rel)
    wk7_items = [WK7(m, rc) for m in BSUM for rc in range(4)] if SK < NB else []
    if SQ:
        wt_items = [WT(m, ft, kt) for m in range(7) for ft in range(4) for kt in range(4)]
    else:
        wt_items = [WT(0, ft, kt) for ft in range(NG) for kt in range(NG)]
    wt_blocks = cfg.get('wt_blocks', (2, 3, 4, 5))
    n_wt = len(wt_items)
    for i in range(NB):
        pitems = [(Pm(i, c, r), []) for c in range(D // PC) for r in range(D // PR)]
        if i == 0:
            plan.append((0.0, pend))
            pend = []
            side = [L(1, 0), issue(8)] + [L(1, c) for c in range(1, NLC)]
            if SK <= 1:
                side += wk7_items
                wk7_items = []
            spread(pitems, side)
            spread(k_items(1), [L(2, c) for c in range(NLC)])
        elif i + 1 < NB:
            kk = k_items(i + 1)
            nfill = cfg.get('nfill', 2) if i + 1 >= SK else 1
            spread(kk[:nfill], [])
            side = []
            if i + 2 < NB:
                side += [L(i + 2, c) for c in range(NLC)]
            if wk7_items and i + 2 == SK:
                side += wk7_items
                wk7_items = []
            spread(pitems, side)
            side = []
            if i in wt_blocks:
                k_ = wt_blocks.index(i)
                nb_ = len(wt_blocks)
                side = wt_items[n_wt * k_ // nb_:n_wt * (k_ + 1) // nb_]
            spread(kk[nfill:], side)
        else:
            nq0 = cfg.get('nq0', 2)
            spread([(QT(0, 0, m), []) for m in range(nq0)], [])
            spread(pitems, [])
    assert not wk7_items
    n_p1 = len(plan)

    pend = pend + [ZT(g) for g in range(NG)]
    NM = 7 if SQ else 4
    NOm = 7 if SO else 4

    def emit(main, wgt, after, nshare=None):
        nonlocal pend
        if nshare is None or not pend:
            plan.append((wgt, [main] + pend))
            pend = list(after)
        else:
            plan.append((wgt, [main] + pend[:nshare]))
            pend = pend[nshare:] + list(after)

    def q_chunk(i, c, skip=0):
        wq_ = QC * 128 * (HD if SQ else D) / (256.0 * 128 * 1024)
        for m in range(skip, NM):
            after = []
            if SQ:
                after = [GA(i, c, b) for b in range(4) if ST_LAST[b] == m]
                if m == NM - 1:
                    after += [GS(i, c, mm) for mm in range(NOm)]
            else:
                after = [GA(i, c, m)] + ([GS(i, c, mm) for mm in range(NOm)] if m == NM - 1 else [])
            emit(QT(i, c, m), wq_, after, cfg.get('nshare', 2))

    def o_chunk(i, j):
        wo_ = TH * 128 * (HD if SO else D) / (256.0 * 128 * 1024)
        for m in range(NOm):
            if SO:
                after = [E(i, j, b) for b in range(4) if ST_LAST[b] == m]
            else:
                after = [E(i, j, m)]
            emit(O(i, j, m), wo_, after, cfg.get('nshare', 2))

    qitems = [(i, c) for i in range(NB) for c in range(NQ)]
    q_chunk(0, 0, skip=cfg.get('nq0', 2))
    qdone = 1
    n_pre = cfg.get('n_pre', 1)
    for ic in qitems[1:1 + n_pre]:
        q_chunk(*ic)
        qdone += 1
    kv0 = len(plan)
    gs = [0, 4, 1, 5, 2, 6, 3, 7] if SO else list(range(NG))
    kvm = [KV(gs[0])]
    for k_ in range(NG):
        if k_ + 1 < NG:
            kvm.append(KV(gs[k_ + 1]))
        kvm.append(MM(gs[k_]))
    for it in kvm:
        emit(it, cfg.get('w_kvm', 0.5), [], 2)
    rest = qitems[qdone:]
    oitems = [(i, j) for i in range(NB) for j in range(4)]
    lead = cfg.get('lead', NQ + 1)
    y_deadline = None
    for n, (i, j) in enumerate(oitems):
        while rest and qdone < lead + n * NQ // 4:
            q_chunk(*rest.pop(0))
            qdone += 1
        assert (not rest) or qdone >= (i + 1) * NQ + 1
        if not rest and j == 0 and i == NB - 1:
            plan.append((0.0, pend))
            pend = []
        if i == NB - 1 and j == 0:
            y_deadline = len(plan)
        o_chunk(i, j)
    assert not rest
    plan.append((0.0, pend))

    plan[:kv0 + 1] = [(0.0, it_) for _, it_ in plan[:kv0 + 1]]
    tot_w = sum(w for w, _ in plan[:y_deadline])
    acc_w = 0.0
    k = 0
    for j in range(y_deadline):
        w, items = plan[j]
        acc_w += w
        tgt = int(round(len(moe) * acc_w / tot_w))
        while k < tgt:
            items.append(moe[k])
            k += 1
    assert k == len(moe)

    for f in pro:
        f()
    for j, (_, items) in enumerate(plan):
        st['cur'] = j
        for f in items:
            f()

    pltpu.make_async_copy(o_v.at[pl.ds(0, (NB - 1) * TM), :], o_v.at[pl.ds(0, (NB - 1) * TM), :],
                          osem.at[0]).wait()
    idx, y = st['idx'], st['y']
    idx_s = idx[0, 0]
    base = jnp.where(idx_s < (NB - 1) * TM, (idx_s // 16) * 16, 0)
    base = pl.multiple_of(jnp.clip(base, 0, S - 16), 16)
    o16 = o_v[pl.ds(base, 16), :].astype(F32)
    rows16 = lax.broadcasted_iota(jnp.int32, (16, 1), 0) + base
    fix_v[...] = (o16 + jnp.where(rows16 == idx, y, 0.0)).astype(BF16)
    fix_c = pltpu.make_async_copy(fix_v, o_hbm.at[pl.ds(base, 16), :], fsem)
    fix_c.start()
    pltpu.make_async_copy(o_v.at[pl.ds((NB - 1) * TM, TM), :], o_v.at[pl.ds((NB - 1) * TM, TM), :],
                          osem.at[1]).wait()
    fix_c.wait()


def make(TM=256, LNR=32, **cfg):
    @jax.jit
    def kern(A_x, A_wqkv, A_wo, B_x, B_w_r, B_w_gate, B_w_up, B_w_down):
        del B_x
        B, S, D = A_x.shape
        F = B_w_gate.shape[1]
        assert B == 1
        x2 = A_x.reshape(S, D)
        wr2 = B_w_r.reshape(D // 128, 128)
        HD = D // 2
        SQ, SO = cfg.get('SQ', 1), cfg.get('SO', 1)

        any_spec = pl.BlockSpec(memory_space=pl.ANY)
        cp = dict(vmem_limit_bytes=120 * 1024 * 1024)
        if cfg.get('flags'):
            cp['flags'] = cfg['flags']
        out = pl.pallas_call(
            functools.partial(_fused_kernel, S=S, D=D, F=F, TM=TM, LNR=LNR, cfg=cfg),
            out_shape=jax.ShapeDtypeStruct((S, D), BF16),
            in_specs=[any_spec] * 7,
            out_specs=any_spec,
            scratch_shapes=[
                pltpu.VMEM((S, D), BF16),
                pltpu.VMEM((S // 2, D), U32),
                pltpu.VMEM((D, D), BF16),
                pltpu.VMEM((D, D), BF16),
                pltpu.VMEM((2, D, D), BF16),
                pltpu.VMEM((2, D, F), BF16),
                pltpu.VMEM((F, D), BF16),
                pltpu.VMEM((D, D), F32),
                pltpu.VMEM((7, HD // 2, HD), U32) if SO else pltpu.VMEM((2, HD // 2, D), U32),
                pltpu.VMEM((S, D), BF16),
                pltpu.VMEM((2, D, TM), BF16),
                pltpu.VMEM((7, S // 4, HD), U32) if SO else pltpu.VMEM((2, S // 2, HD), U32),
                pltpu.VMEM((7, HD // 2, HD), U32) if SQ else pltpu.VMEM((2, D // 2, HD), U32),
                pltpu.VMEM((D, 128), F32),
                pltpu.VMEM((D, 128), F32),
                pltpu.VMEM((F, 128), F32),
                pltpu.VMEM((5, S // 4, HD), U32),
                pltpu.VMEM((5, HD // 2, HD), U32),
                pltpu.VMEM((16, D), BF16),
                pltpu.VMEM((D // 128, 128), BF16),
                pltpu.SemaphoreType.DMA((4,)),
                pltpu.SemaphoreType.DMA((8,)),
                pltpu.SemaphoreType.DMA((4,)),
                pltpu.SemaphoreType.DMA((2,)),
                pltpu.SemaphoreType.DMA,
                pltpu.SemaphoreType.DMA,
            ],
            compiler_params=pltpu.CompilerParams(**cp),
        )(x2, A_wqkv, A_wo, wr2, B_w_gate, B_w_up, B_w_down)
        return out.reshape(B, S, D)
    return kern


pallas_parallel_sum__linear_attn_block__moe_arch_mod__prompt_kernel = make(
    SQ=1, SO=1, SK=8, RK=128, tie=6)
```

```python
import functools

import jax
import jax.numpy as jnp
from jax import lax
import jax.experimental.pallas as pl
import jax.experimental.pallas.tpu as pltpu

F32 = jnp.float32
BF16 = jnp.bfloat16
U32 = jnp.uint32

HEADS = 32
LN_EPS = 1e-5
PHI_EPS = 1e-6
TM = 256
LNR = 32
PC = 512
QC = 256
EC, EK = 512, 128
TIE = 6
WK_PANEL = 256
X_GROUPS = ((0, 1), (1, 2), (2, 4), (4, 8))
NT_DIMS = (((1,), (1,)), ((), ()))

ST_A = (((0, 1), (3, 1)), ((2, 1), (3, 1)), ((0, 1),), ((3, 1),),
        ((0, 1), (1, 1)), ((2, 1), (0, -1)), ((1, 1), (3, -1)))
ST_B = (((0, 1), (3, 1)), ((0, 1),), ((1, 1), (3, -1)), ((2, 1), (0, -1)),
        ((3, 1),), ((0, 1), (1, 1)), ((2, 1), (3, 1)))
ST_C = (((0, 1), (3, 1)), ((2, 1), (3, -1)), ((1, 1), (3, 1)), ((0, 1), (2, 1)),
        ((0, -1), (1, 1)), ((3, 1),), ((0, 1),))
ST_LAST = (6, 4, 3, 5)
A_SUMS = tuple(m for m in range(7) if len(ST_A[m]) > 1)


def _phi(t):
    return jnp.where(t > 0, t + 1.0, jnp.exp(t)) + PHI_EPS


def _rnd(t):
    return t.astype(BF16).astype(F32)


def _pk(t):
    return pltpu.bitcast(t, U32)


def _upk(t):
    return pltpu.bitcast(t, BF16)


def _comb(blocks, terms):
    out = None
    for b, sign in terms:
        if out is None:
            out = blocks[b] if sign > 0 else -blocks[b]
        else:
            out = out + blocks[b] if sign > 0 else out - blocks[b]
    return out


def _cols(g, w=128):
    return slice(g * w, (g + 1) * w)


def _kernel(x_hbm, wqkv_hbm, wo_hbm, wr_hbm, wg_hbm, wu_hbm, wd_hbm, o_hbm,
            x_v, xn_v, wq_v, wk_v, wvo_v, wgu_v, wd_v, p_v, m7_v, o_v, pk_v, a7_v, wqt_v,
            zc_v, xb_v, hb_v, xs_v, fix_v, wr_v,
            xsem, ksem, wsem, osem, fsem, rsem, *, S, D, F):
    NB = S // TM
    NG = D // 128
    DH = D // HEADS
    HD = D // 2
    TH = TM // 2
    HM, PH = TM // 2, TH // 2
    NLC = TM // LNR
    NQ = HD // QC
    NP = D // WK_PANEL
    wv_v, wo_v = wvo_v.at[0], wvo_v.at[1]
    wg_v, wu_v = wgu_v.at[0], wgu_v.at[1]

    def x_copy(j):
        lo, hi = X_GROUPS[j]
        rs = pl.ds(lo * TM, (hi - lo) * TM)
        return pltpu.make_async_copy(x_hbm.at[rs, :], x_v.at[rs, :], xsem.at[j])

    def wk_copy(j):
        return pltpu.make_async_copy(wqkv_hbm.at[:, pl.ds(D + j * WK_PANEL, WK_PANEL)],
                                     wk_v.at[:, pl.ds(j * WK_PANEL, WK_PANEL)], ksem.at[j])

    def o_copy(i):
        rs = pl.ds(i * TM, TM)
        return pltpu.make_async_copy(o_v.at[rs, :], o_hbm.at[rs, :], osem.at[0])

    def o_strip_copy(g):
        rs, cs = pl.ds((NB - 1) * TM, TM), pl.ds(g * 128, 128)
        return pltpu.make_async_copy(o_v.at[rs, cs], o_hbm.at[rs, cs], osem.at[1])

    wr_c = pltpu.make_async_copy(wr_hbm, wr_v, rsem)
    wq_c = pltpu.make_async_copy(wqkv_hbm.at[:, pl.ds(0, D)], wq_v, wsem.at[0])
    wv_c = pltpu.make_async_copy(wqkv_hbm.at[:, pl.ds(2 * D, D)], wv_v, wsem.at[1])
    wo_c = pltpu.make_async_copy(wo_hbm, wo_v, wsem.at[1])
    wvo_all = pltpu.make_async_copy(wvo_v, wvo_v, wsem.at[1])
    wg_c = pltpu.make_async_copy(wg_hbm, wg_v, wsem.at[2])
    wu_c = pltpu.make_async_copy(wu_hbm, wu_v, wsem.at[2])
    wgu_all = pltpu.make_async_copy(wgu_v, wgu_v, wsem.at[2])
    wd_c = pltpu.make_async_copy(wd_hbm, wd_v, wsem.at[3])

    first = [wr_c, x_copy(0)] + [wk_copy(j) for j in range(NP)] + [x_copy(1)]

    def start_first(k, carry):
        for j, cp in enumerate(first):
            pl.when(k == j)(cp.start)
        return carry

    lax.fori_loop(0, len(first), start_first, 0)

    def start_late(g):
        def f():
            if g == 2:
                x_copy(2).start()
            elif g == 4:
                x_copy(3).start()
            elif g == 6:
                wq_c.start()
            elif g == 8:
                for cp in (wv_c, wo_c, wg_c, wu_c, wd_c):
                    cp.start()
        return f

    wr_c.wait()
    wr8 = wr_v[...].astype(F32)
    wr = jnp.concatenate([wr8[j:j + 1, :] for j in range(NG)], axis=-1)
    zero = lax.shift_right_logical(
        lax.bitcast_convert_type(jnp.abs(wr8[0:1, 0:1]), jnp.int32), 31)[0, 0]

    st = {'best': jnp.full((LNR, 1), -jnp.inf, F32),
          'bidx': jnp.zeros((LNR, 1), jnp.int32),
          'z': [jnp.zeros((8, 128), F32) for _ in range(NG)]}

    def xn_operand(i, m):
        if len(ST_A[m]) == 1:
            b = ST_A[m][0][0]
            r0 = i * HM + (b // 2) * PH
            return xn_v[r0:r0 + PH, _cols(b % 2, HD)]
        return xs_v[A_SUMS.index(m), i * PH:(i + 1) * PH, :]

    def add_product(key, m, val):
        for c, sign in ST_C[m]:
            k = key + (c,)
            if k in st:
                st[k] = st[k] + val if sign > 0 else st[k] - val
            else:
                st[k] = val if sign > 0 else -val

    def LN(i, c):
        def f():
            if c == 0:
                for j, (lo, _) in enumerate(X_GROUPS):
                    if lo == i:
                        x_copy(j).wait()
                if i == 4:
                    wq_c.wait()
            r0 = i * TM + c * LNR
            x = x_v[r0:r0 + LNR, :].astype(F32)
            xc = x - jnp.mean(x, axis=-1, keepdims=True)
            var = jnp.mean(xc * xc, axis=-1, keepdims=True)
            inv = 1.0 / _rnd(jnp.sqrt(_rnd(_rnd(var) + LN_EPS)))
            xn = xc * inv
            xn_v[r0 // 2:(r0 + LNR) // 2, :] = _pk(xn.astype(BF16))
            if c * LNR >= TH:
                r1 = r0 - TH
                top = _upk(xn_v[r1 // 2:(r1 + LNR) // 2, :]).astype(F32)
                blk = (top[:, :HD], top[:, HD:], xn[:, :HD], xn[:, HD:])
                q0 = i * PH + (c * LNR - TH) // 2
                for k, m in enumerate(A_SUMS):
                    xs_v[k, q0:q0 + LNR // 2, :] = _pk(_comb(blk, ST_A[m]).astype(BF16))
            score = jnp.sum(xc * wr, axis=-1, keepdims=True) * inv
            better = score > st['best']
            st['best'] = jnp.where(better, score, st['best'])
            st['bidx'] = jnp.where(
                better, lax.broadcasted_iota(jnp.int32, (LNR, 1), 0) + r0, st['bidx'])
        return f

    def K(i, g):
        def f():
            if i == 0 and (g * 128) % WK_PANEL == 0:
                wk_copy(g * 128 // WK_PANEL).wait()
            st['k', i, g] = jnp.dot(_upk(xn_v[i * HM:(i + 1) * HM, :]), wk_v[:, _cols(g)],
                                    preferred_element_type=F32)
        return f

    def PHIK(i, g):
        def f():
            pk = _phi(st.pop(('k', i, g)))
            acc = st['z'][g]
            for r in range(TM // 8):
                acc = acc + pk[r * 8:(r + 1) * 8, :]
            st['z'][g] = acc
            pk_v[i % 2, _cols(g), :] = pk.T.astype(BF16)
        return f

    def P(i, c):
        def f():
            cs = _cols(c, PC)
            pp = jnp.dot(pk_v[i % 2], _upk(xn_v[i * HM:(i + 1) * HM, cs]),
                         preferred_element_type=F32)
            if i == 0:
                p_v[:, cs] = pp
            else:
                p_v[:, cs] += pp
        return f

    def WT(m, ft, kt):
        def f():
            blk = {b: wq_v[_cols((b // 2) * 4 + kt), _cols((b % 2) * 4 + ft)].astype(F32)
                   for b, _ in ST_B[m]}
            rs = pl.ds(pl.multiple_of(ft * 64 + zero, 64), 64)
            wqt_v[m, rs, _cols(kt)] = _pk(_comb(blk, ST_B[m]).T.astype(BF16))
        return f

    def tie_to(value):
        st.setdefault(('tie', st['cur'] + TIE), []).append(value)

    def tie(raw):
        ties = st.pop(('tie', st['cur']), None)
        if not ties:
            return raw
        t = functools.reduce(lambda a, b: a + b, ties)
        tile = jnp.where(zero != 0, lax.bitcast_convert_type(t, U32), raw[0:8, 0:128])
        top = jnp.concatenate([tile, raw[0:8, 128:]], axis=1)
        return jnp.concatenate([top, raw[8:, :]], axis=0)

    def SELECT():
        def f():
            gmax = jnp.max(st['best'], axis=0, keepdims=True)
            idx = jnp.min(jnp.where(st['best'] == gmax, st['bidx'], S - 1), axis=0, keepdims=True)
            st['gmax'], st['idx'] = gmax, idx
            base = jnp.clip((idx[0, 0] // 16) * 16, 0, S - 16)
            xs = _upk(xn_v[pl.ds(pl.multiple_of(base // 2, 8), 8), :]).astype(F32)
            rows = lax.broadcasted_iota(jnp.int32, (16, 1), 0) + base
            st['xsel'] = jnp.sum(jnp.where(rows == idx, xs, 0.0), axis=0, keepdims=True)
        return f

    def XCOL(g):
        def f():
            xb_v[_cols(g), :] = jnp.broadcast_to(st['xsel'][:, _cols(g)], (128, 128)).T
        return f

    def MATVEC(key, w_v, col_v, c, k0):
        def f():
            acc = None if k0 == 0 else st.pop(key)
            for r in range(k0, k0 + EK, 8):
                w = w_v[r:r + 8, _cols(c, EC)].astype(F32)
                t = w * jnp.concatenate([col_v[r:r + 8, :]] * (EC // 128), axis=-1)
                acc = t if acc is None else acc + t
            st[key] = acc
            tie_to(functools.reduce(lambda a, b: a + b,
                                    [acc[:, _cols(j)] for j in range(EC // 128)]))
        return f

    def SWIGLU(c):
        def f():
            g = jnp.sum(st.pop(('g', c)), axis=0, keepdims=True)
            u = jnp.sum(st.pop(('u', c)), axis=0, keepdims=True)
            h = g * jax.nn.sigmoid(g) * u
            for j in range(EC // 128):
                hcol = jnp.broadcast_to(h[:, _cols(j)], (128, 128)).T
                hb_v[_cols(c * (EC // 128) + j), :] = hcol
            tie_to(hcol[0:8, :])
        return f

    def YOUT():
        def f():
            ys = [jnp.sum(st.pop(('y', c)), axis=0, keepdims=True) for c in range(D // EC)]
            st['y'] = jnp.concatenate(ys, axis=-1) * jax.nn.sigmoid(st['gmax'])
        return f

    expert = [SELECT()] + [XCOL(g) for g in range(NG)]
    for c in range(F // EC):
        expert += [MATVEC(('g', c), wg_v, xb_v, c, k0) for k0 in range(0, D, EK)]
        expert += [MATVEC(('u', c), wu_v, xb_v, c, k0) for k0 in range(0, D, EK)]
        expert.append(SWIGLU(c))
    for c in range(D // EC):
        expert += [MATVEC(('y', c), wd_v, hb_v, c, k0) for k0 in range(0, F, EK)]
    expert.append(YOUT())

    same_head = (lax.broadcasted_iota(jnp.int32, (128, 128), 0) // DH
                 == lax.broadcasted_iota(jnp.int32, (128, 128), 1) // DH)

    def ZCOL(g):
        def f():
            z = jnp.sum(st['z'][g], axis=0, keepdims=True)
            zc_v[_cols(g), :] = jnp.broadcast_to(z, (128, 128)).T
        return f

    def KV(g):
        def f():
            if g == 0:
                wvo_all.wait()
                wgu_all.wait()
                wd_c.wait()
            kv = jnp.dot(p_v[_cols(g), :].astype(BF16), wv_v[:, _cols(g)],
                         preferred_element_type=F32)
            st['kv', g] = jnp.where(same_head, kv, 0.0).astype(BF16)
        return f

    def M(g):
        def f():
            st['m', g] = jnp.dot(st.pop(('kv', g)), wo_v[_cols(g), :], preferred_element_type=F32)
            if g >= 4:
                top, bot = st.pop(('m', g - 4)), st.pop(('m', g))
                blk = (top[:, :HD], top[:, HD:], bot[:, :HD], bot[:, HD:])
                for m in range(7):
                    m7_v[m, _cols(g - 4, 64), :] = _pk(_comb(blk, ST_B[m]).astype(BF16))
        return f

    def QT(i, c, m):
        def f():
            lhs = _upk(tie(wqt_v[m, _cols(c, QC // 2), :]))
            add_product(('q', i, c), m, lax.dot_general(
                lhs, _upk(xn_operand(i, m)), NT_DIMS, preferred_element_type=F32))
        return f

    def NORM(i, c, b):
        def f():
            q = st.pop(('q', i, c, b))
            f0 = (b % 2) * HD + c * QC
            outs = []
            for h in range(0, QC, DH):
                pq = _phi(q[h:h + DH, :])
                t = pq * zc_v[f0 + h:f0 + h + DH, :]
                s = (t[0:8] + t[8:16]) + (t[16:24] + t[24:32])
                outs.append(pq * (1.0 / (jnp.sum(s, axis=0, keepdims=True) + PHI_EPS)))
            st['a', i, c, b] = jnp.concatenate(outs, axis=0)
        return f

    def AOP(i, c, m):
        def f():
            blk = {b: st['a', i, c, b] for b in range(4)}
            a7_v[m, i * PH:(i + 1) * PH, _cols(c, QC)] = _pk(_comb(blk, ST_A[m]).T.astype(BF16))
        return f

    def O(i, j, m):
        def f():
            lhs = _upk(tie(a7_v[m, i * PH:(i + 1) * PH, :]))
            add_product(('o', i, j), m, jnp.dot(lhs, _upk(m7_v[m, :, _cols(j)]),
                                                preferred_element_type=F32))
        return f

    def OUT(i, j, b):
        def f():
            att = st.pop(('o', i, j, b))
            g = (b % 2) * 4 + j
            r0 = i * TM + (b // 2) * TH
            out = (x_v[r0:r0 + TH, _cols(g)].astype(F32)
                   + _upk(xn_v[r0 // 2:(r0 + TH) // 2, _cols(g)]).astype(F32) + att)
            if i == NB - 1:
                rows = lax.broadcasted_iota(jnp.int32, (TH, 1), 0) + r0
                out = out + jnp.where(rows == st['idx'], st['y'][:, _cols(g)], 0.0)
            o_v[r0:r0 + TH, _cols(g)] = out.astype(BF16)
            done = st.setdefault(('done', i), set())
            done.add((j, b))
            if i == NB - 1:
                if (j, b % 2) in done and (j, 2 + b % 2) in done:
                    o_strip_copy(g).start()
            elif len(done) == 16:
                o_copy(i).start()
        return f

    plan, pend = [], []

    def emit(mains, side=(), weight=0.0, share=None):
        nonlocal pend
        for j, (main, released) in enumerate(mains):
            now = pend if share is None else pend[:share]
            lo, hi = len(side) * j // len(mains), len(side) * (j + 1) // len(mains)
            plan.append((weight, [main] + now + list(side[lo:hi])))
            pend = pend[len(now):] + list(released)

    def k_items(i):
        return [(K(i, g), [PHIK(i, g)]) for g in range(NG)]

    def ln_items(i):
        return [LN(i, c) for c in range(NLC)]

    def q_items(i, c, ms):
        out = []
        for m in ms:
            rel = [NORM(i, c, b) for b in range(4) if ST_LAST[b] == m]
            out.append((QT(i, c, m), rel + [AOP(i, c, mm) for mm in range(7)] * (m == 6)))
        return out

    wt = [WT(m, ft, kt) for m in range(7) for ft in range(4) for kt in range(4)]
    for g, (main, released) in enumerate(k_items(0)):
        plan.append((0.0, [main, start_late(g)] + pend))
        pend = released
    plan.append((0.0, pend))
    pend = []
    ln1 = ln_items(1)
    emit([(P(0, c), []) for c in range(D // PC)], [ln1[0], start_late(8)] + ln1[1:])
    emit(k_items(1), ln_items(2))
    for i in range(1, NB - 1):
        ks = k_items(i + 1)
        emit(ks[:1])
        emit([(P(i, c), []) for c in range(D // PC)], ln_items(i + 2) if i + 2 < NB else ())
        emit(ks[1:], wt[len(wt) * (i - 2) // 4:len(wt) * (i - 1) // 4] if 2 <= i < 6 else ())
    emit(q_items(0, 0, range(2)))
    emit([(P(NB - 1, c), []) for c in range(D // PC)])

    pend = pend + [ZCOL(g) for g in range(NG)]
    wq_ = QC * 128 * HD / (256.0 * 128 * 1024)
    wo_ = TH * 128 * HD / (256.0 * 128 * 1024)
    qs = [(i, c) for i in range(NB) for c in range(NQ)]
    emit(q_items(0, 0, range(2, 7)), share=2)
    emit(q_items(*qs[1], range(7)), share=2)
    qs, qdone = qs[2:], 2
    order = [0, 4, 1, 5, 2, 6, 3, 7]
    emit([(KV(order[0]), [])])
    for k, g in enumerate(order):
        emit([(KV(h), []) for h in order[k + 1:k + 2]] + [(M(g), [])], weight=0.5, share=2)
    deadline = None
    for n, (i, j) in enumerate((i, j) for i in range(NB) for j in range(4)):
        while qs and qdone < NQ + 1 + n * NQ // 4:
            emit(q_items(*qs.pop(0), range(7)), weight=wq_, share=2)
            qdone += 1
        if i == NB - 1 and j == 0:
            plan.append((0.0, pend))
            pend = []
            deadline = len(plan)
        emit([(O(i, j, m), [OUT(i, j, b) for b in range(4) if ST_LAST[b] == m]) for m in range(7)],
             weight=wo_, share=2)
    plan.append((0.0, pend))

    total, acc, k = sum(w for w, _ in plan[:deadline]), 0.0, 0
    for w, items in plan[:deadline]:
        acc += w
        while k < int(round(len(expert) * acc / total)):
            items.append(expert[k])
            k += 1
    assert k == len(expert) and not qs

    for f in ln_items(0):
        f()
    for j, (_, items) in enumerate(plan):
        st['cur'] = j
        for f in items:
            f()

    early = pl.ds(0, (NB - 1) * TM)
    pltpu.make_async_copy(o_v.at[early, :], o_v.at[early, :], osem.at[0]).wait()
    idx = st['idx']
    base = jnp.where(idx[0, 0] < (NB - 1) * TM, (idx[0, 0] // 16) * 16, 0)
    base = pl.multiple_of(jnp.clip(base, 0, S - 16), 16)
    rows = lax.broadcasted_iota(jnp.int32, (16, 1), 0) + base
    fix_v[...] = (o_v[pl.ds(base, 16), :].astype(F32)
                  + jnp.where(rows == idx, st['y'], 0.0)).astype(BF16)
    fix_c = pltpu.make_async_copy(fix_v, o_hbm.at[pl.ds(base, 16), :], fsem)
    fix_c.start()
    last = pl.ds((NB - 1) * TM, TM)
    pltpu.make_async_copy(o_v.at[last, :], o_v.at[last, :], osem.at[1]).wait()
    fix_c.wait()


@jax.jit
def pallas_parallel_sum__linear_attn_block__moe_arch_mod__prompt_kernel(
    A_x: jax.Array,
    A_wqkv: jax.Array,
    A_wo: jax.Array,
    B_x: jax.Array,
    B_w_r: jax.Array,
    B_w_gate: jax.Array,
    B_w_up: jax.Array,
    B_w_down: jax.Array,
):
    del B_x
    B, S, D = A_x.shape
    F = B_w_gate.shape[1]
    assert B == 1 and S == 8 * TM and D == 1024 and F % EC == 0
    HD = D // 2
    any_spec = pl.BlockSpec(memory_space=pl.ANY)
    out = pl.pallas_call(
        functools.partial(_kernel, S=S, D=D, F=F),
        out_shape=jax.ShapeDtypeStruct((S, D), BF16),
        in_specs=[any_spec] * 7,
        out_specs=any_spec,
        scratch_shapes=[
            pltpu.VMEM((S, D), BF16),
            pltpu.VMEM((S // 2, D), U32),
            pltpu.VMEM((D, D), BF16),
            pltpu.VMEM((D, D), BF16),
            pltpu.VMEM((2, D, D), BF16),
            pltpu.VMEM((2, D, F), BF16),
            pltpu.VMEM((F, D), BF16),
            pltpu.VMEM((D, D), F32),
            pltpu.VMEM((7, HD // 2, HD), U32),
            pltpu.VMEM((S, D), BF16),
            pltpu.VMEM((2, D, TM), BF16),
            pltpu.VMEM((7, S // 4, HD), U32),
            pltpu.VMEM((7, HD // 2, HD), U32),
            pltpu.VMEM((D, 128), F32),
            pltpu.VMEM((D, 128), F32),
            pltpu.VMEM((F, 128), F32),
            pltpu.VMEM((5, S // 4, HD), U32),
            pltpu.VMEM((16, D), BF16),
            pltpu.VMEM((D // 128, 128), BF16),
            pltpu.SemaphoreType.DMA((len(X_GROUPS),)),
            pltpu.SemaphoreType.DMA((D // WK_PANEL,)),
            pltpu.SemaphoreType.DMA((4,)),
            pltpu.SemaphoreType.DMA((2,)),
            pltpu.SemaphoreType.DMA,
            pltpu.SemaphoreType.DMA,
        ],
        compiler_params=pltpu.CompilerParams(vmem_limit_bytes=120 * 1024 * 1024),
    )(A_x.reshape(S, D), A_wqkv, A_wo, B_w_r.reshape(D // 128, 128), B_w_gate, B_w_up, B_w_down)
    return out.reshape(B, S, D)
```
